```python
import os as _os
_os.environ.setdefault("JAX_PLATFORMS", "cpu")
import jax
import jax.numpy as jnp

def _softmax(x, axis=-1):
    return jax.nn.softmax(x, axis=axis)
def _gelu(x):
    return jax.nn.gelu(x, approximate=True)
def _silu(x):
    return jax.nn.silu(x)
def _sigmoid(x):
    return jax.nn.sigmoid(x)
def _layernorm(x, axis=-1, eps=1e-5):
    m = jnp.mean(x, axis=axis, keepdims=True)
    v = jnp.var(x, axis=axis, keepdims=True)
    return (x - m) / jnp.sqrt(v + eps)
def _scatter_add(tgt, idx, src, axis=0):
    return tgt.at[idx].add(src)
def _segment_sum(src, seg, n):
    return jax.ops.segment_sum(src, seg, n)
class _Rng:
    def __init__(self, key):
        self._k = key
    def _next(self):
        self._k, sub = jax.random.split(self._k)
        return sub
    def normal(self, shape):
        return jax.random.normal(self._next(), shape, dtype=jnp.bfloat16)
    def randint(self, lo, hi, shape):
        return jax.random.randint(self._next(), shape, lo, hi, dtype=jnp.int32)
    def uniform(self, shape, lo=0.0, hi=1.0):
        return jax.random.uniform(self._next(), shape, jnp.bfloat16, lo, hi)
    def permutation(self, n):
        return jax.random.permutation(self._next(), n)


kernel_name = 'standalone__mha_block_cached__near_ridge'

def setup_inputs():
    _rng = _Rng(jax.random.key(int.from_bytes(__import__("os").urandom(4), "little")))
    _w = (lambda a: (lambda t: t.astype(jnp.bfloat16) if jnp.issubdtype(t.dtype, jnp.floating) else t)(jnp.asarray(a)))
    B, Sq, D = 8, 144, 448
    H, Sk, Dh = 16, 2048, 256
    return {
        "x": _w((lambda *s: _rng.normal(s) * 0.8)(B, Sq, D)),
        "k_cache": _w((lambda *s: _rng.normal(s) * 0.8)(B, H, Sk, Dh)),
        "v_cache": _w((lambda *s: _rng.normal(s) * 0.05)(B, H, Sk, Dh)),
        "wq": _w((lambda *s: _rng.normal(s) * 0.8)(D, H * Dh) * (D ** -0.5)),
        "wo": _w((lambda *s: _rng.normal(s) * 0.05)(H * Dh, D) * ((H * Dh) ** -0.5)),
    }

def reference(x, k_cache, v_cache, wq, wo):
    B, Sq, D = x.shape
    H, Dh = 16, 256
    q = (lambda x, *d: x.transpose(*d))((x @ wq).reshape(B, Sq, H, Dh), 0, 2, 1, 3)
    scores = jnp.einsum("bhqd,bhkd->bhqk", q, k_cache) * (Dh ** -0.5)
    p = _softmax(scores, axis=-1)
    o = jnp.einsum("bhqk,bhkd->bhqd", p, v_cache)
    return (lambda x, *d: x.transpose(*d))(o, 0, 2, 1, 3).reshape(B, Sq, H * Dh) @ wo
```

```python
import jax
import jax.numpy as jnp
from jax import lax
import jax.experimental.pallas as pl
import jax.experimental.pallas.tpu as pltpu

H, DH = 16, 256
NT = (((1,), (1,)), ((), ()))

def slide(S, P=64):
    per = 2048 // P // S
    return [(a, (S - 1 - j) * per + c, j) for c in range(per) for a in (0, 1) for j in range(S)]
def w1(order, dk=0):
    return [((c // 32), c % 32, dk if c < 32 else 0) for c in order]
M11 = [(i * 11) % 64 for i in range(64)]

def make(lanes=None, L=2, rot=0, cuts=(16, 16, 16, 16, 0), P=64, wchunk=True, pred='lane', flags=None, compute=True, extra_slots=0):
    lanes = lanes or slide(4)
    NL = len(lanes)
    assert sum(cuts) == NL
    dmax = max(l[2] for l in lanes)
    nslot = L + dmax + 1 + (1 if rot else 0) + extra_slots

    def fn(x, k_cache, v_cache, wq, wo):
        B, Sq, D = x.shape
        Sk = k_cache.shape[2]
        n = B * H

        def kern(x_hbm, k_hbm, v_hbm, wq_hbm, wot_hbm, out_hbm,
                 xbuf, wqbuf, wobuf, kv, acc, obuf, sem):
            XS, WQS, WOS, OS = 2 * nslot, 2 * nslot + 1, 2 * nslot + 2, 2 * nslot + 3
            def lane(u, t, guard):
                a, c, d = lanes[u]
                hd = t + d
                src = k_hbm if a == 0 else v_hbm
                s = hd % nslot if isinstance(hd, int) else lax.rem(hd, nslot)
                def go():
                    row = hd * Sk + c * P
                    if not isinstance(row, int): row = pl.multiple_of(row, P)
                    pltpu.make_async_copy(src.at[pl.ds(row, P)], kv.at[2 * s + a, pl.ds(c * P, P)], sem.at[2 * s + a]).start(priority=u % 2)
                if guard: pl.when(hd < n)(go)
                else: go()
            def o_cp(b): return pltpu.make_async_copy(obuf.at[b], out_hbm.at[b], sem.at[OS + b])

            wcps = []
            if wchunk:
                for b in range(B):
                    for r in range(0, Sq, 48):
                        wcps.append(pltpu.make_async_copy(x_hbm.at[b, pl.ds(r, 48)], xbuf.at[b, pl.ds(r, 48)], sem.at[XS]))
                for sm, src, dst in ((WQS, wq_hbm, wqbuf), (WOS, wot_hbm, wobuf)):
                    for r in range(0, D, 16):
                        for c in range(0, H * DH, 1024):
                            wcps.append(pltpu.make_async_copy(src.at[pl.ds(r, 16), pl.ds(c, 1024)], dst.at[pl.ds(r, 16), pl.ds(c, 1024)], sem.at[sm]))
            else:
                wcps = [pltpu.make_async_copy(x_hbm, xbuf, sem.at[XS]), pltpu.make_async_copy(wq_hbm, wqbuf, sem.at[WQS]), pltpu.make_async_copy(wot_hbm, wobuf, sem.at[WOS])]
            for j, c in enumerate(wcps): c.start(priority=j % 2)
            for t in range(-dmax, L + 1):
                for u in range(NL if t < L else rot):
                    if t + lanes[u][2] >= 0: lane(u, t, False)
            pltpu.make_async_copy(xbuf, xbuf, sem.at[XS]).wait()
            pltpu.make_async_copy(wqbuf, wqbuf, sem.at[WQS]).wait()
            pltpu.make_async_copy(wobuf, wobuf, sem.at[WOS]).wait()

            def body(i, guard):
                b = i // H; h = i % H
                s = lax.rem(i, nslot)
                pos = [0]
                def issue(cnt):
                    for p in range(pos[0], pos[0] + cnt):
                        u = p + rot
                        lane(u % NL, i + L + u // NL, guard)
                    pos[0] += cnt
                pltpu.make_async_copy(kv.at[2 * s], kv.at[2 * s], sem.at[2 * s]).wait()
                pltpu.make_async_copy(kv.at[2 * s + 1], kv.at[2 * s + 1], sem.at[2 * s + 1]).wait()
                issue(cuts[0])
                hs = pl.ds(pl.multiple_of(h * DH, DH), DH)
                if compute:
                    q = jnp.dot(xbuf[b], wqbuf[:, hs], preferred_element_type=jnp.float32)
                    q = q.astype(jnp.bfloat16) * jnp.bfloat16(DH ** -0.5)
                    issue(cuts[1])
                    sc = lax.dot_general(q, kv[2 * s], NT, preferred_element_type=jnp.float32)
                    issue(cuts[2])
                    m = jnp.max(sc, axis=-1, keepdims=True)
                    p = jnp.exp(sc - m)
                    l = jnp.sum(p, axis=-1, keepdims=True)
                    issue(cuts[3])
                    o = jnp.dot(p.astype(jnp.bfloat16), kv[2 * s + 1], preferred_element_type=jnp.float32)
                    issue(cuts[4])
                    o = (o / l).astype(jnp.bfloat16)
                    y = lax.dot_general(o, wobuf[:, hs], NT, preferred_element_type=jnp.float32)
                else:
                    issue(sum(cuts[1:]))
                    y = (kv[2 * s, :Sq, :] + kv[2 * s + 1, :Sq, :]).astype(jnp.float32)
                    y = jnp.concatenate([y, y[:, :D - DH]], axis=1)
                y = y + jnp.where(h > 0, acc[...], 0.0)
                acc[...] = y
                @pl.when(h == H - 1)
                def _():
                    obuf[b] = acc[...].astype(obuf.dtype)
                    o_cp(b).start()
            if pred == 'lane':
                lax.fori_loop(0, n, lambda i, _: body(i, True), None)
            else:
                nmain = n - (L + dmax + (1 if rot else 0))
                lax.fori_loop(0, nmain, lambda i, _: body(i, False), None)
                lax.fori_loop(nmain, n, lambda i, _: body(i, True), None)
            for b in range(B): o_cp(b).wait()

        return pl.pallas_call(
            kern,
            in_specs=[pl.BlockSpec(memory_space=pltpu.HBM)] * 5,
            out_specs=pl.BlockSpec(memory_space=pltpu.HBM),
            out_shape=jax.ShapeDtypeStruct((B, Sq, D), x.dtype),
            scratch_shapes=[
                pltpu.VMEM((B, Sq, D), jnp.bfloat16),
                pltpu.VMEM((D, H * DH), jnp.bfloat16),
                pltpu.VMEM((D, H * DH), jnp.bfloat16),
                pltpu.VMEM((2 * nslot, Sk, DH), jnp.bfloat16),
                pltpu.VMEM((Sq, D), jnp.float32),
                pltpu.VMEM((B, Sq, D), jnp.bfloat16),
                pltpu.SemaphoreType.DMA((2 * nslot + 3 + B,)),
            ],
            compiler_params=pltpu.CompilerParams(vmem_limit_bytes=100 * 1024 * 1024, disable_bounds_checks=True, flags=flags),
        )(x, k_cache.reshape(B * H * Sk, DH), v_cache.reshape(B * H * Sk, DH), wq, wo.T)
    return fn


_impl = make(w1(M11), L=2, rot=16, cuts=(64,0,0,0,0), pred='split')

@jax.jit
def pallas_standalone__mha_block_cached__near_ridge_kernel(x, k_cache, v_cache, wq, wo):
    return _impl(x, k_cache, v_cache, wq, wo)
```

```python
import jax
import jax.numpy as jnp
from jax import lax
import jax.experimental.pallas as pl
import jax.experimental.pallas.tpu as pltpu

H, DH = 16, 256
NT = (((1,), (1,)), ((), ()))

def make(oK=10, oV=6, mK=7, mV=8, sK=(), sV=(), nq=8, nv=8, flags=None, owhen='vwait', ochunk=32, oq=None,
         nb=None, dbg=None, compute=True, order='bh', nosem=False, scopes=False, skipq=False):
    P = 64
    qi, vi = 32 // nq, 32 // nv
    nK = nV = 4
    offs = (oK, oV); ms = (mK, mV); skips = (tuple(sK), tuple(sV))

    def where(a, hs, k, n):
        t, up = hs >> 2, (hs >> 1) & 1
        c4, d, hf = (hs & 1) * 2 + (k >> 2), (k >> 1) & 1, k & 1
        t1 = n - ms[a]
        if t < t1: return t + d, hf * 16 + (t & 1) * 8 + up * 4 + c4
        return t + up, hf * 16 + (up ^ (t1 % 2)) * 8 + 2 * c4 + d

    def simulate(n):
        seen = set(); occupant = {}; consumed = set()
        def sim(a, hs, k):
            hd, ch = where(a, hs, k, n)
            if 0 <= hd < n:
                assert (a, hd, ch) not in seen, ("dup", a, hd, ch)
                seen.add((a, hd, ch))
                prev = occupant.get((a, hd % 4))
                assert prev is None or prev == hd or (a, prev) in consumed, ("WAR", a, hd, prev)
                occupant[(a, hd % 4)] = hd
        def sim_wait(a, hd): assert all((a, hd, ch) in seen for ch in range(32)), ("deadlock", a, hd)
        for a in (0, 1):
            for hs in range(-4, offs[a]):
                for k in range(8): sim(a, hs, k)
        for j in range(-1, n):
            for half in (0, 1):
                act = (j + 1 < n) if half == 0 else (j >= 0)
                if not act: continue
                sim_wait(half, j + 1 - half)
                if j >= 0:
                    for g in (4 * j + 2 * half, 4 * j + 2 * half + 1):
                      for k in range(8):
                        for a in (0, 1):
                            sk = [4 * n - s for s in skips[a]]
                            if g not in sk: sim(a, g + offs[a] - sum(g > s for s in sk), k)
                consumed.add((half, j + 1 - half))
        assert len(seen) == 64 * n, "missing"
    simulate((nb or 8) * H)

    def fn(x, k_cache, v_cache, wq, wo):
        B, Sq, D = x.shape
        Sk = k_cache.shape[2]
        BB = nb or B
        n = BB * H

        def kern(x_hbm, k_hbm, v_hbm, wq_hbm, wot_hbm, out_hbm,
                 xbuf, wqbuf, wobuf, kv, acc, qbuf, mbuf, sbuf, obuf, sem):
            XS, WQS, WOS, OS, FS = [nK + nV + j for j in range(5)]
            def bh(j):
                if order == 'bh': return j >> 4, j & (H - 1)
                return j & (BB - 1), j >> (BB.bit_length() - 1)
            def slot(a, hd): return a * nK + (hd & 3)
            def start(a, hd, chunk, prio):
                s = slot(a, hd)
                src = k_hbm if a == 0 else v_hbm
                r0 = pl.multiple_of(chunk * P, P)
                b_, h_ = bh(hd)
                row = pl.multiple_of((hd if order == 'bh' else b_ * H + h_) * Sk + r0, P)
                pltpu.make_async_copy(src.at[pl.ds(row, P)], kv.at[s, pl.ds(r0, P)], sem.at[s]).start(priority=prio)
            def wait(a, hd):
                s = slot(a, hd)
                if scopes:
                    with jax.named_scope("kw" if a == 0 else "vw"):
                        pltpu.make_async_copy(kv.at[s], kv.at[s], sem.at[s]).wait()
                else:
                    pltpu.make_async_copy(kv.at[s], kv.at[s], sem.at[s]).wait()
            def fetch(a, hs, k, prio, ok=None):
                t, up = hs >> 2, (hs >> 1) & 1
                c4, d, hf = (hs & 1) * 2 + (k >> 2), (k >> 1) & 1, k & 1
                t1 = n - ms[a]
                hd, ch = t + d, hf * 16 + (t & 1) * 8 + up * 4 + c4
                if ms[a]:
                    h2, c2 = t + up, hf * 16 + (up ^ (t1 % 2)) * 8 + 2 * c4 + d
                    hd = jnp.where(t < t1, hd, h2); ch = jnp.where(t < t1, ch, c2)
                cond = (hd >= 0) & (hd < n)
                if ok is not None: cond = cond & ok
                pl.when(cond)(lambda: start(a, hd, ch, prio))
            def issuer(g):
                st = {}
                for a in (0, 1):
                  for e in (0, 1):
                    gg = 2 * g + e
                    hs, ok = gg + offs[a], gg >= 0
                    for s in skips[a]:
                        hs = hs - (gg > 4 * n - s).astype(jnp.int32)
                        ok = ok & (gg != 4 * n - s)
                    st[a, e] = (hs, ok)
                def issue(u0, cnt):
                    for u in range(u0, u0 + cnt):
                        hs, ok = st[u % 2, u // 16]
                        fetch(u % 2, hs, (u // 2) % 8, u % 2, ok)
                return issue
            def brows(b): return pl.ds(b * Sq if isinstance(b, int) else pl.multiple_of(b * Sq, 16), Sq)
            def hcols(h): return pl.ds(h * DH if isinstance(h, int) else pl.multiple_of(h * DH, DH), DH)

            def wround(c, _):
                r8 = (c // 2) * 8; c0 = pl.multiple_of((c % 2) * 2048, 2048)
                for j in range(D // 64):
                    sl = (pl.ds(pl.multiple_of(64 * j + r8, 8), 8), pl.ds(c0, 2048))
                    pltpu.make_async_copy(wq_hbm.at[sl], wqbuf.at[sl], sem.at[WQS]).start(priority=0)
                    pltpu.make_async_copy(wot_hbm.at[sl], wobuf.at[sl], sem.at[WOS]).start(priority=1)
                for j in range(2):
                    rs = pl.ds(pl.multiple_of((16 * j + c) * 32, 32), 32)
                    pltpu.make_async_copy(x_hbm.at[rs], xbuf.at[rs], sem.at[XS]).start(priority=j)
            lax.fori_loop(0, 16, wround, None)
            for j in range(32, B * Sq // 32):
                pltpu.make_async_copy(x_hbm.at[pl.ds(j * 32, 32)], xbuf.at[pl.ds(j * 32, 32)], sem.at[XS]).start(priority=j % 2)
            lead = oK - oV
            def konly(r, _):
                for e in range(2): fetch(0, (r >> 2) - 4, (r & 3) * 2 + e, e)
            lax.fori_loop(0, 4 * lead, konly, None)
            def both(r, _):
                fetch(0, (r >> 3) - 4 + lead, r & 7, 0)
                fetch(1, (r >> 3) - 4, r & 7, 1)
            lax.fori_loop(0, 8 * (oV + 4), both, None)
            acc[...] = jnp.zeros_like(acc)
            pltpu.make_async_copy(xbuf, xbuf, sem.at[XS]).wait()
            pltpu.make_async_copy(wqbuf, wqbuf, sem.at[WQS]).wait()
            pltpu.make_async_copy(wobuf, wobuf, sem.at[WOS]).wait()
            def qproj(i):
                b, h = bh(i)
                q = jnp.dot(xbuf[brows(b), :], wqbuf[:, hcols(h)], preferred_element_type=jnp.float32)
                qbuf[...] = q.astype(jnp.bfloat16) * jnp.bfloat16(DH ** -0.5)
            qproj(0)

            nlate = 1 if order == 'bh' or owhen in ('vpre', 'vwait') else 2
            nearly = (BB - nlate) * Sq
            def early_start(cond):
                if not ochunk:
                    rs = pl.ds(0, nearly)
                    pl.when(cond)(lambda: pltpu.make_async_copy(obuf.at[rs], out_hbm.at[rs], sem.at[OS]).start(priority=oq or 0))
                    return
                assert nearly % (2 * ochunk) == 0
                def one(r, _):
                    for e in range(2):
                        rs = pl.ds(pl.multiple_of((2 * r + e) * ochunk, 8), ochunk)
                        pltpu.make_async_copy(obuf.at[rs], out_hbm.at[rs], sem.at[OS]).start(priority=e)
                lax.fori_loop(0, jnp.where(cond, nearly // (2 * ochunk), 0), one, None)

            def body(i, _):
                j = i - 1
                @pl.when(i < n)
                def _():
                    wait(0, i)
                    issue = issuer(2 * j)
                    s = slot(0, i)
                    if not compute: return issue(0, 32)
                    q = qbuf[...]
                    kc = Sk // nq
                    mrun = None
                    for c in range(nq):
                        sc = lax.dot_general(q, kv[s, pl.ds(c * kc, kc), :], NT, preferred_element_type=jnp.float32)
                        for r in range(kc // 128):
                            t = sc[:, r * 128:(r + 1) * 128]
                            mrun = t if mrun is None else jnp.maximum(mrun, t)
                        sbuf[i & 1, :, c * kc:(c + 1) * kc] = sc
                        issue(c * qi, qi)
                    mbuf[i & 1] = jnp.broadcast_to(jnp.max(mrun, axis=-1, keepdims=True), mrun.shape)
                    if skipq: pl.when(i + 1 < n)(lambda: qproj(i + 1))
                    else: qproj(jnp.minimum(i + 1, n - 1))
                @pl.when(j >= 0)
                def _():
                    if owhen == 'vpre': early_start(j == n - 1)
                    if owhen == 'vpre2': early_start(j == n - 2)
                    wait(1, j)
                    if owhen == 'vwait': early_start(j == n - 1)
                    if owhen == 'vwait2': early_start(j == n - 2)
                    issue = issuer(2 * j + 1)
                    s = slot(1, j)
                    if not compute: return issue(0, 32)
                    b, h = bh(j)
                    mx = mbuf[j & 1]
                    vc = Sk // nv
                    o = lrun = None
                    for c in range(nv):
                        ps = []
                        for r in range(vc // 128):
                            t = jnp.exp(sbuf[j & 1, :, c * vc + r * 128:c * vc + (r + 1) * 128] - mx)
                            lrun = t if lrun is None else lrun + t
                            ps.append(t.astype(jnp.bfloat16))
                        p = jnp.concatenate(ps, axis=1) if len(ps) > 1 else ps[0]
                        oc = jnp.dot(p, kv[s, pl.ds(c * vc, vc), :], preferred_element_type=jnp.float32)
                        o = oc if o is None else o + oc
                        issue(c * vi, vi)
                        if owhen == ('pv2', c): early_start(j == n - 2)
                    on = (o * (1.0 / jnp.sum(lrun, axis=-1, keepdims=True))).astype(jnp.bfloat16)
                    y = lax.dot_general(on, wobuf[:, hcols(h)], NT, preferred_element_type=jnp.float32)
                    if order == 'bh':
                        y = y + jnp.where(h > 0, acc[...], 0.0)
                        acc[...] = y
                    else:
                        y = y + acc[brows(b), :]
                        acc[brows(b), :] = y
                    obuf[brows(b), :] = y.astype(obuf.dtype)
            lax.fori_loop(0, n + 1, body, None)

            if (not compute and not owhen) or dbg == 'nofin': return
            late = pl.ds(nearly, nlate * Sq)
            fin = pltpu.make_async_copy(obuf.at[late], out_hbm.at[late], sem.at[FS])
            with jax.named_scope("fin"): fin.start()
            if owhen:
                rs = pl.ds(0, nearly)
                with jax.named_scope("pro"): pltpu.make_async_copy(obuf.at[rs], out_hbm.at[rs], sem.at[OS]).wait()
            with jax.named_scope("fin"): fin.wait()

        out = pl.pallas_call(
            kern,
            in_specs=[pl.BlockSpec(memory_space=pltpu.HBM)] * 5,
            out_specs=pl.BlockSpec(memory_space=pltpu.HBM),
            out_shape=jax.ShapeDtypeStruct((B * Sq, D), x.dtype),
            scratch_shapes=[
                pltpu.VMEM((B * Sq, D), jnp.bfloat16),
                pltpu.VMEM((D, H * DH), jnp.bfloat16),
                pltpu.VMEM((D, H * DH), jnp.bfloat16),
                pltpu.VMEM((nK + nV, Sk, DH), jnp.bfloat16),
                pltpu.VMEM((Sq if order == 'bh' else B * Sq, D), jnp.float32),
                pltpu.VMEM((Sq, DH), jnp.bfloat16),
                pltpu.VMEM((2, Sq, 128), jnp.float32),
                pltpu.VMEM((2, Sq, Sk), jnp.float32),
                pltpu.VMEM((B * Sq, D), jnp.bfloat16),
                pltpu.SemaphoreType.DMA((nK + nV + 5,)),
            ],
            compiler_params=pltpu.CompilerParams(vmem_limit_bytes=100 * 1024 * 1024, disable_bounds_checks=True, disable_semaphore_checks=nosem, flags=flags),
        )(x.reshape(B * Sq, D), k_cache.reshape(B * H * Sk, DH), v_cache.reshape(B * H * Sk, DH), wq, wo.T)
        return out.reshape(B, Sq, D)
    return fn


_impl = make(mK=4, mV=6, sK=(18,), nosem=True, owhen=('pv2', 6), ochunk=0, oq=1)

@jax.jit
def pallas_standalone__mha_block_cached__near_ridge_kernel(x, k_cache, v_cache, wq, wo):
    return _impl(x, k_cache, v_cache, wq, wo)
```

```python
import numpy as np

import jax
import jax.numpy as jnp
from jax import lax
import jax.experimental.pallas as pl
import jax.experimental.pallas.tpu as pltpu

_H = 16
_DH = 256
_ROWS = 64
_CHUNKS = 32
_RING = 8
_SPLIT = 8
_PER_SPLIT = 32 // _SPLIT
_WARMUP = 256
_NT = (((1,), (1,)), ((), ()))


def _fetch_order(n, narrow, single, phase):
    order = []

    def pieces(todo):
        for c in range(4):
            for head, half, quarter in todo:
                order.append((head, half * 16 + (quarter + phase) % 4 * 4 + c))

    def chunk(half, eighth, c):
        return half * 16 + (eighth * 8 + c + 4 * phase) % 16

    for head in range(-3, n - narrow):
        quarter = (head - (n - narrow)) % 4
        pieces([(head + d, half, quarter) for half in range(2) for d in range(4)])
    head = n - narrow
    pieces([
        (head, 0, 0), (head + 1, 0, 0), (head + 2, 0, 2), (head + 1, 1, 1),
        (head, 1, 0), (head + 1, 0, 1), (head + 2, 1, 2), (head + 1, 1, 0),
    ])
    eighth = 0
    for head in range(n - narrow + 2, n):
        if head < n - single:
            for c in range(8):
                for d in range(2):
                    for half in range(2):
                        order.append((head + d, chunk(half, eighth, c)))
            eighth = 1 - eighth
        else:
            for d in range(2):
                for c in range(8):
                    for half in range(2):
                        order.append((head + d, chunk(half, eighth ^ d, c)))
    return order


def _copy_schedule(n):
    orders = (_fetch_order(n, 17, 3, 0), _fetch_order(n, 13, 6, 2))
    lead = (3 * _CHUNKS + 80, 3 * _CHUNKS + 48)
    pauses = ((62, 58, 54, 50, 22), (44, 37, 30, 23))
    batches = n // _H
    issued = [0, 0]

    def take(a):
        i = issued[a]
        issued[a] += 1
        if i >= len(orders[a]) or not 0 <= orders[a][i][0] < n:
            return -1
        head, c = orders[a][i]
        place = (head % batches) * _H + head // batches
        return (place * _CHUNKS + c) | (head % _RING) << 12 | a << 20

    warmup = []
    while issued[0] < lead[0] or issued[1] < lead[1]:
        entry = take(0 if lead[0] - issued[0] >= lead[1] - issued[1] else 1)
        if entry >= 0:
            warmup.append(entry)
    loop = []
    for quarter in range(-4, 4 * n):
        for _ in range(8):
            for a in range(2):
                runs = quarter >= 0 and quarter // 2 != 2 * n - 2
                loop.append(take(a) if runs and 4 * n - quarter not in pauses[a] else -1)
    table = np.full((-(-(_WARMUP + len(loop)) // 1024) * 1024,), -1, np.int32)
    table[0] = (len(warmup) + 1) // 2
    table[1 : 1 + len(warmup)] = warmup
    table[_WARMUP : _WARMUP + len(loop)] = loop
    copies = table[1:][table[1:] >= 0]
    assert len(warmup) + 2 <= _WARMUP
    assert len(np.unique(copies)) == len(copies) == 2 * _CHUNKS * n
    return table


def _kernel(
    x_hbm, k_hbm, v_hbm, wq_hbm, wot_hbm, table_hbm, out_hbm,
    x_buf, wq_buf, wot_buf, kv_buf, q_buf, s_buf, m_buf, acc, out_buf, table, sem,
):
    sq = q_buf.shape[0]
    sk = kv_buf.shape[1]
    d_model = wq_buf.shape[0]
    batches = x_buf.shape[0] // sq
    n = batches * _H
    keys = sk // _SPLIT
    x_sem, wq_sem, wo_sem, out_sem, table_sem = (sem.at[2 * _RING + i] for i in range(5))

    def batch_rows(i):
        return pl.ds(pl.multiple_of(i % batches * sq, 16), sq)

    def head_cols(i):
        return pl.ds(pl.multiple_of(i // batches * _DH, _DH), _DH)

    def fetch(a, entry, queue):
        slot = a * _RING + ((entry >> 12) & (_RING - 1))
        src = pl.ds(pl.multiple_of((entry & 4095) * _ROWS, _ROWS), _ROWS)
        dst = pl.ds(pl.multiple_of((entry & (_CHUNKS - 1)) * _ROWS, _ROWS), _ROWS)
        pltpu.make_async_copy(
            (k_hbm, v_hbm)[a].at[src], kv_buf.at[slot, dst], sem.at[slot]
        ).start(priority=queue)

    def issue(half_iteration, c):
        for u in range(c * _PER_SPLIT, (c + 1) * _PER_SPLIT):
            entry = table[_WARMUP + half_iteration * 32 + u]
            pl.when(entry >= 0)(lambda: fetch(u % 2, entry, u % 2))

    def arrived(a, i):
        slot = a * _RING + (i & (_RING - 1))
        pltpu.make_async_copy(kv_buf.at[slot], kv_buf.at[slot], sem.at[slot]).wait()
        return slot

    def write_out(first, count, queue):
        rows = pl.ds(first * sq, count * sq)
        pltpu.make_async_copy(out_buf.at[rows], out_hbm.at[rows], out_sem).start(
            priority=queue
        )

    def project_q(i):
        q = jnp.dot(
            x_buf[batch_rows(i), :],
            wq_buf[:, head_cols(i)],
            preferred_element_type=jnp.float32,
        )
        q_buf[...] = q.astype(q_buf.dtype) * (_DH**-0.5)

    table_copy = pltpu.make_async_copy(table_hbm, table, table_sem)
    table_copy.start()

    def fetch_x(block, queue):
        rows = pl.ds(pl.multiple_of(block * 32, 32), 32)
        pltpu.make_async_copy(x_hbm.at[rows], x_buf.at[rows], x_sem).start(priority=queue)

    @pl.loop(0, 16)
    def _(c):
        cols = pl.ds(pl.multiple_of(c % 2 * 2048, 2048), 2048)
        for j in range(d_model // 64):
            rows = pl.ds(pl.multiple_of(64 * j + c // 2 * 8, 8), 8)
            pltpu.make_async_copy(
                wq_hbm.at[rows, cols], wq_buf.at[rows, cols], wq_sem
            ).start(priority=0)
            pltpu.make_async_copy(
                wot_hbm.at[rows, cols], wot_buf.at[rows, cols], wo_sem
            ).start(priority=1)
        for queue in range(2):
            fetch_x(16 * queue + c, queue)

    @pl.loop(16, x_buf.shape[0] // 64)
    def _(c):
        for queue in range(2):
            fetch_x(2 * c + queue, queue)

    acc[...] = jnp.zeros_like(acc)
    table_copy.wait()

    @pl.loop(0, table[0])
    def _(r):
        for queue in range(2):
            entry = table[1 + 2 * r + queue]
            for a in range(2):
                pl.when((entry >> 20) == a)(lambda: fetch(a, entry, queue))

    pltpu.make_async_copy(x_buf, x_buf, x_sem).wait()
    pltpu.make_async_copy(wq_buf, wq_buf, wq_sem).wait()
    pltpu.make_async_copy(wot_buf, wot_buf, wo_sem).wait()
    project_q(jnp.int32(0))

    @pl.loop(0, n + 1)
    def _(i):
        @pl.when(i < n)
        def _():
            slot = arrived(0, i)
            q = q_buf[...]
            top = None
            for c in range(_SPLIT):
                s = lax.dot_general(
                    q, kv_buf[slot, pl.ds(c * keys, keys), :], _NT,
                    preferred_element_type=jnp.float32,
                )
                for r in range(0, keys, 128):
                    part = s[:, r : r + 128]
                    top = part if top is None else jnp.maximum(top, part)
                s_buf[i & 1, :, c * keys : (c + 1) * keys] = s
                issue(2 * i, c)
            m_buf[i & 1] = jnp.broadcast_to(
                jnp.max(top, axis=-1, keepdims=True), top.shape
            )
            project_q(jnp.minimum(i + 1, n - 1))

        @pl.when(i > 0)
        def _():
            j = i - 1
            slot = arrived(1, j)
            m = m_buf[j & 1]
            o = total = None
            for c in range(_SPLIT):
                p = []
                for r in range(c * keys, (c + 1) * keys, 128):
                    e = jnp.exp(s_buf[j & 1, :, r : r + 128] - m)
                    total = e if total is None else total + e
                    p.append(e.astype(kv_buf.dtype))
                part = jnp.dot(
                    jnp.concatenate(p, axis=1),
                    kv_buf[slot, pl.ds(c * keys, keys), :],
                    preferred_element_type=jnp.float32,
                )
                o = part if o is None else o + part
                issue(2 * i + 1, c)
                if c == _SPLIT - 2:
                    pl.when(j == n - 2)(lambda: write_out(0, batches - 2, 1))
            o = o * (1.0 / jnp.sum(total, axis=-1, keepdims=True))
            y = lax.dot_general(
                o.astype(wot_buf.dtype), wot_buf[:, head_cols(j)], _NT,
                preferred_element_type=jnp.float32,
            )
            y = y + acc[batch_rows(j), :]
            acc[batch_rows(j), :] = y
            out_buf[batch_rows(j), :] = y.astype(out_buf.dtype)
            pl.when(j == n - 2)(lambda: write_out(batches - 2, 1, 1))

    write_out(batches - 1, 1, 0)
    pltpu.make_async_copy(out_buf, out_hbm, out_sem).wait()


@jax.jit
def pallas_standalone__mha_block_cached__near_ridge_kernel(
    x: jax.Array,
    k_cache: jax.Array,
    v_cache: jax.Array,
    wq: jax.Array,
    wo: jax.Array,
):
    b, sq, d_model = x.shape
    sk = k_cache.shape[2]
    assert k_cache.shape == v_cache.shape == (b, _H, _ROWS * _CHUNKS, _DH)
    schedule = _copy_schedule(b * _H)
    hbm = pl.BlockSpec(memory_space=pltpu.HBM)

    out = pl.pallas_call(
        _kernel,
        in_specs=[hbm] * 6,
        out_specs=hbm,
        out_shape=jax.ShapeDtypeStruct((b * sq, d_model), x.dtype),
        scratch_shapes=[
            pltpu.VMEM((b * sq, d_model), x.dtype),
            pltpu.VMEM((d_model, _H * _DH), wq.dtype),
            pltpu.VMEM((d_model, _H * _DH), wo.dtype),
            pltpu.VMEM((2 * _RING, sk, _DH), k_cache.dtype),
            pltpu.VMEM((sq, _DH), x.dtype),
            pltpu.VMEM((2, sq, sk), jnp.float32),
            pltpu.VMEM((2, sq, 128), jnp.float32),
            pltpu.VMEM((b * sq, d_model), jnp.float32),
            pltpu.VMEM((b * sq, d_model), x.dtype),
            pltpu.SMEM(schedule.shape, jnp.int32),
            pltpu.SemaphoreType.DMA((2 * _RING + 5,)),
        ],
        compiler_params=pltpu.CompilerParams(
            vmem_limit_bytes=64 * 1024 * 1024,
            disable_bounds_checks=True,
            disable_semaphore_checks=True,
        ),
    )(
        x.reshape(b * sq, d_model),
        k_cache.reshape(b * _H * sk, _DH),
        v_cache.reshape(b * _H * sk, _DH),
        wq,
        wo.T,
        schedule,
    )
    return out.reshape(b, sq, d_model)
```

```python
import numpy as np

import jax
import jax.numpy as jnp
from jax import lax
import jax.experimental.pallas as pl
import jax.experimental.pallas.tpu as pltpu

_H = 16
_DH = 256
_ROWS = 64
_CHUNKS = 32
_RING = 8
_SPLIT = 8
_PER_SPLIT = 32 // _SPLIT
_WARMUP = 256
_NT = (((1,), (1,)), ((), ()))


def _fetch_order(n, narrow, single, phase):
    order = []

    def pieces(todo):
        for c in range(4):
            for head, half, quarter in todo:
                order.append((head, half * 16 + (quarter + phase) % 4 * 4 + c))

    def chunk(half, eighth, c):
        return half * 16 + (eighth * 8 + c + 4 * phase) % 16

    for head in range(-3, n - narrow):
        quarter = (head - (n - narrow)) % 4
        pieces([(head + d, half, quarter) for half in range(2) for d in range(4)])
    head = n - narrow
    pieces([
        (head, 0, 0), (head + 1, 0, 0), (head + 2, 0, 2), (head + 1, 1, 1),
        (head, 1, 0), (head + 1, 0, 1), (head + 2, 1, 2), (head + 1, 1, 0),
    ])
    eighth = 0
    for head in range(n - narrow + 2, n):
        if head < n - single:
            for c in range(8):
                for d in range(2):
                    for half in range(2):
                        order.append((head + d, chunk(half, eighth, c)))
            eighth = 1 - eighth
        else:
            for d in range(2):
                for c in range(8):
                    for half in range(2):
                        order.append((head + d, chunk(half, eighth ^ d, c)))
    return order


def _copy_schedule(n):
    orders = (_fetch_order(n, 17, 3, 0), _fetch_order(n, 13, 6, 2))
    lead = (3 * _CHUNKS + 80, 3 * _CHUNKS + 48)
    pauses = ((62, 58, 54, 50, 22), (44, 37, 30, 23))
    batches = n // _H
    issued = [0, 0]

    def take(a):
        i = issued[a]
        issued[a] += 1
        if i >= len(orders[a]) or not 0 <= orders[a][i][0] < n:
            return -1
        head, c = orders[a][i]
        place = (head % batches) * _H + head // batches
        return (place * _CHUNKS + c) | (head % _RING) << 12 | a << 20

    warmup = []
    while issued[0] < lead[0] or issued[1] < lead[1]:
        entry = take(0 if lead[0] - issued[0] >= lead[1] - issued[1] else 1)
        if entry >= 0:
            warmup.append(entry)
    loop = []
    for quarter in range(-4, 4 * n):
        for _ in range(8):
            for a in range(2):
                runs = quarter >= 0 and quarter // 2 != 2 * n - 2
                loop.append(take(a) if runs and 4 * n - quarter not in pauses[a] else -1)
    table = np.full((-(-(_WARMUP + len(loop)) // 1024) * 1024,), -1, np.int32)
    table[0] = (len(warmup) + 1) // 2
    table[1 : 1 + len(warmup)] = warmup
    table[_WARMUP : _WARMUP + len(loop)] = loop
    copies = table[1:][table[1:] >= 0]
    assert len(warmup) + 2 <= _WARMUP
    assert len(np.unique(copies)) == len(copies) == 2 * _CHUNKS * n
    return table


def _kernel(
    x_hbm, k_hbm, v_hbm, wq_hbm, wot_hbm, table_hbm, out_hbm,
    x_buf, wq_buf, wot_buf, kv_buf, q_buf, s_buf, m_buf, acc, out_buf, table, sem,
):
    sq = q_buf.shape[0]
    sk = kv_buf.shape[1]
    d_model = wq_buf.shape[0]
    batches = x_buf.shape[0] // sq
    n = batches * _H
    keys = sk // _SPLIT
    x_sem, wq_sem, wo_sem, out_sem, table_sem = (sem.at[2 * _RING + i] for i in range(5))

    def batch_rows(i):
        first = i % batches * sq
        return pl.ds(first if isinstance(i, int) else pl.multiple_of(first, 16), sq)

    def head_cols(i):
        first = i // batches * _DH
        return pl.ds(first if isinstance(i, int) else pl.multiple_of(first, _DH), _DH)

    def fetch(a, entry, queue):
        slot = a * _RING + ((entry >> 12) & (_RING - 1))
        src = pl.ds(pl.multiple_of((entry & 4095) * _ROWS, _ROWS), _ROWS)
        dst = pl.ds(pl.multiple_of((entry & (_CHUNKS - 1)) * _ROWS, _ROWS), _ROWS)
        pltpu.make_async_copy(
            (k_hbm, v_hbm)[a].at[src], kv_buf.at[slot, dst], sem.at[slot]
        ).start(priority=queue)

    def issue(half_iteration, c):
        for u in range(c * _PER_SPLIT, (c + 1) * _PER_SPLIT):
            entry = table[_WARMUP + half_iteration * 32 + u]
            pl.when(entry >= 0)(lambda: fetch(u % 2, entry, u % 2))

    def arrived(a, i):
        slot = a * _RING + (i & (_RING - 1))
        pltpu.make_async_copy(kv_buf.at[slot], kv_buf.at[slot], sem.at[slot]).wait()
        return slot

    def write_out(first, count, queue):
        rows = pl.ds(first * sq, count * sq)
        pltpu.make_async_copy(out_buf.at[rows], out_hbm.at[rows], out_sem).start(
            priority=queue
        )

    def project_q(i):
        q = jnp.dot(
            x_buf[batch_rows(i), :],
            wq_buf[:, head_cols(i)],
            preferred_element_type=jnp.float32,
        )
        q_buf[...] = q.astype(q_buf.dtype) * (_DH**-0.5)

    table_copy = pltpu.make_async_copy(table_hbm, table, table_sem)
    table_copy.start()

    def fetch_x(block, queue):
        rows = pl.ds(pl.multiple_of(block * 32, 32), 32)
        pltpu.make_async_copy(x_hbm.at[rows], x_buf.at[rows], x_sem).start(priority=queue)

    @pl.loop(0, 16)
    def _(c):
        cols = pl.ds(pl.multiple_of(c % 2 * 2048, 2048), 2048)
        for j in range(d_model // 64):
            rows = pl.ds(pl.multiple_of(64 * j + c // 2 * 8, 8), 8)
            pltpu.make_async_copy(
                wq_hbm.at[rows, cols], wq_buf.at[rows, cols], wq_sem
            ).start(priority=0)
            pltpu.make_async_copy(
                wot_hbm.at[rows, cols], wot_buf.at[rows, cols], wo_sem
            ).start(priority=1)
        for queue in range(2):
            fetch_x(16 * queue + c, queue)

    @pl.loop(16, x_buf.shape[0] // 64)
    def _(c):
        for queue in range(2):
            fetch_x(2 * c + queue, queue)

    acc[...] = jnp.zeros_like(acc)
    table_copy.wait()

    @pl.loop(0, table[0])
    def _(r):
        for queue in range(2):
            entry = table[1 + 2 * r + queue]
            for a in range(2):
                pl.when((entry >> 20) == a)(lambda: fetch(a, entry, queue))

    pltpu.make_async_copy(x_buf, x_buf, x_sem).wait()
    pltpu.make_async_copy(wq_buf, wq_buf, wq_sem).wait()
    pltpu.make_async_copy(wot_buf, wot_buf, wo_sem).wait()
    project_q(0)

    @pl.loop(0, n + 1)
    def _(i):
        @pl.when(i < n)
        def _():
            slot = arrived(0, i)
            q = q_buf[...]
            top = None
            for c in range(_SPLIT):
                s = lax.dot_general(
                    q, kv_buf[slot, pl.ds(c * keys, keys), :], _NT,
                    preferred_element_type=jnp.float32,
                )
                for r in range(0, keys, 128):
                    part = s[:, r : r + 128]
                    top = part if top is None else jnp.maximum(top, part)
                s_buf[i & 1, :, c * keys : (c + 1) * keys] = s
                issue(2 * i, c)
            m_buf[i & 1] = jnp.broadcast_to(
                jnp.max(top, axis=-1, keepdims=True), top.shape
            )
            project_q(jnp.minimum(i + 1, n - 1))

        @pl.when(i > 0)
        def _():
            j = i - 1
            slot = arrived(1, j)
            m = m_buf[j & 1]
            o = total = None
            for c in range(_SPLIT):
                p = []
                for r in range(c * keys, (c + 1) * keys, 128):
                    e = jnp.exp(s_buf[j & 1, :, r : r + 128] - m)
                    total = e if total is None else total + e
                    p.append(e.astype(kv_buf.dtype))
                part = jnp.dot(
                    jnp.concatenate(p, axis=1),
                    kv_buf[slot, pl.ds(c * keys, keys), :],
                    preferred_element_type=jnp.float32,
                )
                o = part if o is None else o + part
                issue(2 * i + 1, c)
                if c == _SPLIT - 2:
                    pl.when(j == n - 2)(lambda: write_out(0, batches - 2, 1))
            o = o * (1.0 / jnp.sum(total, axis=-1, keepdims=True))
            y = lax.dot_general(
                o.astype(wot_buf.dtype), wot_buf[:, head_cols(j)], _NT,
                preferred_element_type=jnp.float32,
            )
            y = y + acc[batch_rows(j), :]
            acc[batch_rows(j), :] = y
            out_buf[batch_rows(j), :] = y.astype(out_buf.dtype)
            pl.when(j == n - 2)(lambda: write_out(batches - 2, 1, 1))

    write_out(batches - 1, 1, 0)
    pltpu.make_async_copy(out_buf, out_hbm, out_sem).wait()


@jax.jit
def pallas_standalone__mha_block_cached__near_ridge_kernel(
    x: jax.Array,
    k_cache: jax.Array,
    v_cache: jax.Array,
    wq: jax.Array,
    wo: jax.Array,
):
    b, sq, d_model = x.shape
    sk = k_cache.shape[2]
    assert k_cache.shape == v_cache.shape == (b, _H, _ROWS * _CHUNKS, _DH)
    schedule = _copy_schedule(b * _H)
    hbm = pl.BlockSpec(memory_space=pltpu.HBM)

    out = pl.pallas_call(
        _kernel,
        in_specs=[hbm] * 6,
        out_specs=hbm,
        out_shape=jax.ShapeDtypeStruct((b * sq, d_model), x.dtype),
        scratch_shapes=[
            pltpu.VMEM((b * sq, d_model), x.dtype),
            pltpu.VMEM((d_model, _H * _DH), wq.dtype),
            pltpu.VMEM((d_model, _H * _DH), wo.dtype),
            pltpu.VMEM((2 * _RING, sk, _DH), k_cache.dtype),
            pltpu.VMEM((sq, _DH), x.dtype),
            pltpu.VMEM((2, sq, sk), jnp.float32),
            pltpu.VMEM((2, sq, 128), jnp.float32),
            pltpu.VMEM((b * sq, d_model), jnp.float32),
            pltpu.VMEM((b * sq, d_model), x.dtype),
            pltpu.SMEM(schedule.shape, jnp.int32),
            pltpu.SemaphoreType.DMA((2 * _RING + 5,)),
        ],
        compiler_params=pltpu.CompilerParams(
            vmem_limit_bytes=64 * 1024 * 1024,
            disable_bounds_checks=True,
            disable_semaphore_checks=True,
        ),
    )(
        x.reshape(b * sq, d_model),
        k_cache.reshape(b * _H * sk, _DH),
        v_cache.reshape(b * _H * sk, _DH),
        wq,
        wo.T,
        schedule,
    )
    return out.reshape(b, sq, d_model)
```

```python
import functools

import numpy as np

import jax
import jax.numpy as jnp
from jax import lax
import jax.experimental.pallas as pl
import jax.experimental.pallas.tpu as pltpu

_H = 16
_DH = 256
_ROWS = 64
_CHUNKS = 32
_RING = 8
_SPLIT = 8
_PER_SPLIT = 32 // _SPLIT
_WARMUP = 256
_NT = (((1,), (1,)), ((), ()))


def _fetch_order(n, narrow, single, phase):
    order = []

    def pieces(todo):
        for c in range(4):
            for head, half, quarter in todo:
                order.append((head, half * 16 + (quarter + phase) % 4 * 4 + c))

    def chunk(half, eighth, c):
        return half * 16 + (eighth * 8 + c + 4 * phase) % 16

    for head in range(-3, n - narrow):
        quarter = (head - (n - narrow)) % 4
        pieces([(head + d, half, quarter) for half in range(2) for d in range(4)])
    head = n - narrow
    pieces([
        (head, 0, 0), (head + 1, 0, 0), (head + 2, 0, 2), (head + 1, 1, 1),
        (head, 1, 0), (head + 1, 0, 1), (head + 2, 1, 2), (head + 1, 1, 0),
    ])
    eighth = 0
    for head in range(n - narrow + 2, n):
        if head < n - single:
            for c in range(8):
                for d in range(2):
                    for half in range(2):
                        order.append((head + d, chunk(half, eighth, c)))
            eighth = 1 - eighth
        else:
            for d in range(2):
                for c in range(8):
                    for half in range(2):
                        order.append((head + d, chunk(half, eighth ^ d, c)))
    return order


def _copy_schedule(n):
    orders = (_fetch_order(n, 17, 3, 0), _fetch_order(n, 13, 6, 2))
    lead = (3 * _CHUNKS + 80, 3 * _CHUNKS + 48)
    pauses = ((62, 58, 54, 50, 22), (44, 37, 30, 23))
    batches = n // _H
    issued = [0, 0]

    def take(a):
        i = issued[a]
        issued[a] += 1
        if i >= len(orders[a]) or not 0 <= orders[a][i][0] < n:
            return -1
        head, c = orders[a][i]
        place = (head % batches) * _H + head // batches
        return (place * _CHUNKS + c) | (head % _RING) << 12 | a << 20

    warmup = []
    while issued[0] < lead[0] or issued[1] < lead[1]:
        entry = take(0 if lead[0] - issued[0] >= lead[1] - issued[1] else 1)
        if entry >= 0:
            warmup.append(entry)
    loop = []
    for quarter in range(-4, 4 * n):
        for _ in range(8):
            for a in range(2):
                runs = quarter >= 0 and quarter // 2 != 2 * n - 2
                loop.append(take(a) if runs and 4 * n - quarter not in pauses[a] else -1)
    table = np.full((-(-(_WARMUP + len(loop)) // 1024) * 1024,), -1, np.int32)
    table[: len(warmup)] = warmup
    table[_WARMUP : _WARMUP + len(loop)] = loop
    copies = table[table >= 0]
    assert len(warmup) < _WARMUP
    assert len(np.unique(copies)) == len(copies) == 2 * _CHUNKS * n
    return table, (len(warmup) + 1) // 2


def _kernel(
    x_hbm, k_hbm, v_hbm, wq_hbm, wot_hbm, table_hbm, out_hbm,
    x_buf, wq_buf, wot_buf, kv_buf, q_buf, s_buf, m_buf, acc, out_buf, table, sem,
    *, warmup_pairs,
):
    sq = q_buf.shape[0]
    sk = kv_buf.shape[1]
    d_model = wq_buf.shape[0]
    batches = x_buf.shape[0] // sq
    n = batches * _H
    keys = sk // _SPLIT
    x_sem, wq_sem, wo_sem, out_sem, table_sem = (sem.at[2 * _RING + i] for i in range(5))

    def batch_rows(i):
        first = i % batches * sq
        return pl.ds(first if isinstance(i, int) else pl.multiple_of(first, 16), sq)

    def head_cols(i):
        first = i // batches * _DH
        return pl.ds(first if isinstance(i, int) else pl.multiple_of(first, _DH), _DH)

    def fetch(a, entry, queue):
        slot = a * _RING + ((entry >> 12) & (_RING - 1))
        src = pl.ds(pl.multiple_of((entry & 4095) * _ROWS, _ROWS), _ROWS)
        dst = pl.ds(pl.multiple_of((entry & (_CHUNKS - 1)) * _ROWS, _ROWS), _ROWS)
        pltpu.make_async_copy(
            (k_hbm, v_hbm)[a].at[src], kv_buf.at[slot, dst], sem.at[slot]
        ).start(priority=queue)

    def issue(half_iteration, c):
        for u in range(c * _PER_SPLIT, (c + 1) * _PER_SPLIT):
            entry = table[_WARMUP + half_iteration * 32 + u]
            pl.when(entry >= 0)(lambda: fetch(u % 2, entry, u % 2))

    def arrived(a, i):
        slot = a * _RING + (i & (_RING - 1))
        pltpu.make_async_copy(kv_buf.at[slot], kv_buf.at[slot], sem.at[slot]).wait()
        return slot

    def write_out(first, count, queue):
        rows = pl.ds(first * sq, count * sq)
        pltpu.make_async_copy(out_buf.at[rows], out_hbm.at[rows], out_sem).start(
            priority=queue
        )

    def project_q(i):
        q = jnp.dot(
            x_buf[batch_rows(i), :],
            wq_buf[:, head_cols(i)],
            preferred_element_type=jnp.float32,
        )
        q_buf[...] = q.astype(q_buf.dtype) * (_DH**-0.5)

    table_copy = pltpu.make_async_copy(table_hbm, table, table_sem)
    table_copy.start()

    def fetch_x(block, queue):
        rows = pl.ds(pl.multiple_of(block * 32, 32), 32)
        pltpu.make_async_copy(x_hbm.at[rows], x_buf.at[rows], x_sem).start(priority=queue)

    @pl.loop(0, 16)
    def _(c):
        cols = pl.ds(pl.multiple_of(c % 2 * 2048, 2048), 2048)
        for j in range(d_model // 64):
            rows = pl.ds(pl.multiple_of(64 * j + c // 2 * 8, 8), 8)
            pltpu.make_async_copy(
                wq_hbm.at[rows, cols], wq_buf.at[rows, cols], wq_sem
            ).start(priority=0)
            pltpu.make_async_copy(
                wot_hbm.at[rows, cols], wot_buf.at[rows, cols], wo_sem
            ).start(priority=1)
        for queue in range(2):
            fetch_x(16 * queue + c, queue)

    @pl.loop(16, x_buf.shape[0] // 64)
    def _(c):
        for queue in range(2):
            fetch_x(2 * c + queue, queue)

    acc[...] = jnp.zeros_like(acc)
    table_copy.wait()

    @pl.loop(0, warmup_pairs)
    def _(r):
        for queue in range(2):
            entry = table[2 * r + queue]
            for a in range(2):
                pl.when((entry >> 20) == a)(lambda: fetch(a, entry, queue))

    pltpu.make_async_copy(x_buf, x_buf, x_sem).wait()
    pltpu.make_async_copy(wq_buf, wq_buf, wq_sem).wait()
    pltpu.make_async_copy(wot_buf, wot_buf, wo_sem).wait()
    project_q(0)

    @pl.loop(0, n + 1)
    def _(i):
        @pl.when(i < n)
        def _():
            slot = arrived(0, i)
            q = q_buf[...]
            top = None
            for c in range(_SPLIT):
                s = lax.dot_general(
                    q, kv_buf[slot, pl.ds(c * keys, keys), :], _NT,
                    preferred_element_type=jnp.float32,
                )
                for r in range(0, keys, 128):
                    part = s[:, r : r + 128]
                    top = part if top is None else jnp.maximum(top, part)
                s_buf[i & 1, :, c * keys : (c + 1) * keys] = s
                issue(2 * i, c)
            m_buf[i & 1] = jnp.broadcast_to(
                jnp.max(top, axis=-1, keepdims=True), top.shape
            )
            project_q(jnp.minimum(i + 1, n - 1))

        @pl.when(i > 0)
        def _():
            j = i - 1
            slot = arrived(1, j)
            m = m_buf[j & 1]
            o = total = None
            for c in range(_SPLIT):
                p = []
                for r in range(c * keys, (c + 1) * keys, 128):
                    e = jnp.exp(s_buf[j & 1, :, r : r + 128] - m)
                    total = e if total is None else total + e
                    p.append(e.astype(kv_buf.dtype))
                part = jnp.dot(
                    jnp.concatenate(p, axis=1),
                    kv_buf[slot, pl.ds(c * keys, keys), :],
                    preferred_element_type=jnp.float32,
                )
                o = part if o is None else o + part
                issue(2 * i + 1, c)
                if c == _SPLIT - 2:
                    pl.when(j == n - 2)(lambda: write_out(0, batches - 2, 1))
            o = o * (1.0 / jnp.sum(total, axis=-1, keepdims=True))
            y = lax.dot_general(
                o.astype(wot_buf.dtype), wot_buf[:, head_cols(j)], _NT,
                preferred_element_type=jnp.float32,
            )
            y = y + acc[batch_rows(j), :]
            acc[batch_rows(j), :] = y
            out_buf[batch_rows(j), :] = y.astype(out_buf.dtype)
            pl.when(j == n - 2)(lambda: write_out(batches - 2, 1, 1))

    write_out(batches - 1, 1, 0)
    pltpu.make_async_copy(out_buf, out_hbm, out_sem).wait()


@jax.jit
def pallas_standalone__mha_block_cached__near_ridge_kernel(
    x: jax.Array,
    k_cache: jax.Array,
    v_cache: jax.Array,
    wq: jax.Array,
    wo: jax.Array,
):
    b, sq, d_model = x.shape
    sk = k_cache.shape[2]
    assert k_cache.shape == v_cache.shape == (b, _H, _ROWS * _CHUNKS, _DH)
    schedule, warmup_pairs = _copy_schedule(b * _H)
    hbm = pl.BlockSpec(memory_space=pltpu.HBM)

    out = pl.pallas_call(
        functools.partial(_kernel, warmup_pairs=warmup_pairs),
        in_specs=[hbm] * 6,
        out_specs=hbm,
        out_shape=jax.ShapeDtypeStruct((b * sq, d_model), x.dtype),
        scratch_shapes=[
            pltpu.VMEM((b * sq, d_model), x.dtype),
            pltpu.VMEM((d_model, _H * _DH), wq.dtype),
            pltpu.VMEM((d_model, _H * _DH), wo.dtype),
            pltpu.VMEM((2 * _RING, sk, _DH), k_cache.dtype),
            pltpu.VMEM((sq, _DH), x.dtype),
            pltpu.VMEM((2, sq, sk), jnp.float32),
            pltpu.VMEM((2, sq, 128), jnp.float32),
            pltpu.VMEM((b * sq, d_model), jnp.float32),
            pltpu.VMEM((b * sq, d_model), x.dtype),
            pltpu.SMEM(schedule.shape, jnp.int32),
            pltpu.SemaphoreType.DMA((2 * _RING + 5,)),
        ],
        compiler_params=pltpu.CompilerParams(
            vmem_limit_bytes=64 * 1024 * 1024,
            disable_bounds_checks=True,
            disable_semaphore_checks=True,
        ),
    )(
        x.reshape(b * sq, d_model),
        k_cache.reshape(b * _H * sk, _DH),
        v_cache.reshape(b * _H * sk, _DH),
        wq,
        wo.T,
        schedule,
    )
    return out.reshape(b, sq, d_model)
```
